```python
import jax
import jax.numpy as jnp

def _softmax(x, axis=-1):
    return jax.nn.softmax(x, axis=axis)
def _gelu(x):
    return jax.nn.gelu(x, approximate=True)
def _silu(x):
    return jax.nn.silu(x)
def _sigmoid(x):
    return jax.nn.sigmoid(x)
def _layernorm(x, axis=-1, eps=1e-5):
    m = jnp.mean(x, axis=axis, keepdims=True)
    v = jnp.var(x, axis=axis, keepdims=True)
    return (x - m) / jnp.sqrt(v + eps)
def _scatter_add(tgt, idx, src, axis=0):
    return tgt.at[idx].add(src)
def _segment_sum(src, seg, n):
    return jax.ops.segment_sum(src, seg, n)
class _Rng:
    def __init__(self, key):
        self._k = key
    def _next(self):
        self._k, sub = jax.random.split(self._k)
        return sub
    def normal(self, shape):
        return jax.random.normal(self._next(), shape, dtype=jnp.bfloat16)
    def randint(self, lo, hi, shape):
        return jax.random.randint(self._next(), shape, lo, hi, dtype=jnp.int32)
    def uniform(self, shape, lo=0.0, hi=1.0):
        return jax.random.uniform(self._next(), shape, jnp.bfloat16, lo, hi)
    def permutation(self, n):
        return jax.random.permutation(self._next(), n)


kernel_name = 'gated_mix__sliding_block_cached__glu_gated_swiglu__decode'

def setup_inputs():
    _rng = _Rng(jax.random.key(int.from_bytes(__import__("os").urandom(4), "little")))
    _w = (lambda a: (lambda t: t.astype(jnp.bfloat16) if jnp.issubdtype(t.dtype, jnp.floating) else t)(jnp.asarray(a)))
    def _A_setup():
        B, Sq, D = 1, 1, 640
        Hq, Hkv, Sk, Dh = 32, 32, 32768, 192
        assert Hq % Hkv == 0, (Hq, Hkv)
        return {
            "x": _w((lambda *s: _rng.normal(s) * 0.05)(B, Sq, D)),
            "k_cache": _w((lambda *s: _rng.normal(s) * 0.05)(B, Hkv, Sk, Dh)),
            "v_cache": _w((lambda *s: _rng.normal(s) * 0.05)(B, Hkv, Sk, Dh)),
            "wq": _w((lambda *s: _rng.normal(s) * 0.05)(D, Hq * Dh) * (D ** -0.5)),
            "wo": _w((lambda *s: _rng.normal(s) * 0.05)(Hq * Dh, D) * ((Hq * Dh) ** -0.5)),
        }
    _A_in = _A_setup()

    def _B_setup():
        B, S, D, F = 1, 1, 640, 1536
        return {
            "x": _w((lambda *s: _rng.normal(s) * 0.05)(B, S, D)),
            "w1": _w((lambda *s: _rng.normal(s) * 0.05)(D, F) * (2.0 / D) ** 0.5),
            "w3": _w((lambda *s: _rng.normal(s) * 0.05)(D, F) * (2.0 / D) ** 0.5),
            "w2": _w((lambda *s: _rng.normal(s) * 0.05)(F, D) * (2.0 / F) ** 0.5),
        }
    _B_in = _B_setup()

    return {
        "A_x": _A_in["x"],
        "A_k_cache": _A_in["k_cache"],
        "A_v_cache": _A_in["v_cache"],
        "A_wq": _A_in["wq"],
        "A_wo": _A_in["wo"],
        "B_x": _B_in["x"],
        "B_w1": _B_in["w1"],
        "B_w3": _B_in["w3"],
        "B_w2": _B_in["w2"],
        "gate_w": _w((lambda *s: _rng.normal(s) * 0.05)(640)),
    }

def reference(A_x, A_k_cache, A_v_cache, A_wq, A_wo, B_x, B_w1, B_w3, B_w2, gate_w):
    def _A_ref(x, k_cache, v_cache, wq, wo):
        B, Sq, D = x.shape
        Hq, Dh = 32, 192
        Hkv, Sk = k_cache.shape[1], k_cache.shape[2]
        W = min(4096, max(256, Sk // 4))
        rep = Hq // Hkv
        q = (lambda x, *d: x.transpose(*d))((x @ wq).reshape(B, Sq, Hq, Dh), 0, 2, 1, 3)
        k = jnp.repeat(k_cache[:, :, Sk - W:, :], rep, axis=1)
        v = jnp.repeat(v_cache[:, :, Sk - W:, :], rep, axis=1)
        scores = jnp.einsum("bhqd,bhkd->bhqk", q, k) * (Dh ** -0.5)
        p = _softmax(scores, axis=-1)
        o = jnp.einsum("bhqk,bhkd->bhqd", p, v)
        return (lambda x, *d: x.transpose(*d))(o, 0, 2, 1, 3).reshape(B, Sq, Hq * Dh) @ wo

    def _B_ref(x, w1, w3, w2):
        gate = jnp.einsum("bsd,df->bsf", x, w1)
        up = jnp.einsum("bsd,df->bsf", x, w3)
        h = _silu(gate) * up
        out = jnp.einsum("bsf,fd->bsd", h, w2)
        return out

    x = A_x
    g = _sigmoid((x * gate_w).sum(-1, keepdims=True))
    a = _A_ref(x, A_k_cache, A_v_cache, A_wq, A_wo)
    b = _B_ref(x, B_w1, B_w3, B_w2)
    return g * a + (1 - g) * b
```

```python
import jax
import jax.numpy as jnp
from jax import lax
import jax.experimental.pallas as pl
import jax.experimental.pallas.tpu as pltpu

H = 32
DH = 192
G = 2
NBUF = 3
WQ_CH = 4
WO_CH = 8


@jax.jit
def pallas_gated_mix__sliding_block_cached__glu_gated_swiglu__decode_kernel(
    A_x: jax.Array,
    A_k_cache: jax.Array,
    A_v_cache: jax.Array,
    A_wq: jax.Array,
    A_wo: jax.Array,
    B_x: jax.Array,
    B_w1: jax.Array,
    B_w3: jax.Array,
    B_w2: jax.Array,
    gate_w: jax.Array,
):
    D = A_x.shape[-1]
    F = B_w1.shape[-1]
    SK = A_k_cache.shape[2]
    W = min(4096, max(256, SK // 4))
    HD = H * DH
    GR = G * DH
    NG = H // G
    wq_cols = HD // WQ_CH
    wo_rows = HD // WO_CH
    scale = DH ** -0.5
    bf = jnp.bfloat16
    f32 = jnp.float32

    def kernel(x_hbm, k_hbm, v_hbm, wq_hbm, wo_hbm, w1_hbm, w3_hbm, w2_hbm, gw_hbm, o_ref,
               x_v, gw_v, wq_v, wo_v, w1_v, w3_v, w2_v, kbuf, vbuf, qbd, obd,
               sem_s, sem_wq, sem_wo, sem_f, sem_k, sem_v):
        def cp_x():
            return pltpu.make_async_copy(x_hbm, x_v, sem_s.at[0])

        def cp_gw():
            return pltpu.make_async_copy(gw_hbm, gw_v, sem_s.at[1])

        def cp_wq(i):
            sl = pl.ds(i * wq_cols, wq_cols)
            return pltpu.make_async_copy(wq_hbm.at[:, sl], wq_v.at[:, sl], sem_wq.at[i])

        def cp_wo(i):
            sl = pl.ds(i * wo_rows, wo_rows)
            return pltpu.make_async_copy(wo_hbm.at[sl, :], wo_v.at[sl, :], sem_wo.at[i])

        def cp_w1():
            return pltpu.make_async_copy(w1_hbm, w1_v, sem_f.at[0])

        def cp_w3():
            return pltpu.make_async_copy(w3_hbm, w3_v, sem_f.at[1])

        def cp_w2():
            return pltpu.make_async_copy(w2_hbm, w2_v, sem_f.at[2])

        def cp_k(g, s):
            return pltpu.make_async_copy(
                k_hbm.at[pl.ds(g * GR, GR), pl.ds(SK - W, W)], kbuf.at[s], sem_k.at[s])

        def cp_v(g, s):
            return pltpu.make_async_copy(
                v_hbm.at[pl.ds(g * GR, GR), pl.ds(SK - W, W)], vbuf.at[s], sem_v.at[s])

        cp_x().start()
        cp_gw().start()
        for i in range(WQ_CH):
            cp_wq(i).start()
        cp_w1().start()
        cp_w3().start()
        cp_w2().start()
        for g in range(NBUF):
            cp_k(g, g).start()
            cp_v(g, g).start()

        cp_x().wait()
        cp_gw().wait()
        x = x_v[0]
        x8 = jnp.broadcast_to(x, (8, D))
        gw = gw_v[...].reshape(1, D)
        gate = jax.nn.sigmoid(
            jnp.sum(x.astype(f32) * gw.astype(f32), axis=-1, keepdims=True))

        for i in range(WQ_CH):
            cp_wq(i).wait()
            sl = pl.ds(i * wq_cols, wq_cols)
            q = jnp.dot(x8, wq_v[:, sl], preferred_element_type=f32)
            col = lax.broadcasted_iota(jnp.int32, (8, wq_cols), 1) + i * wq_cols
            row = lax.broadcasted_iota(jnp.int32, (8, wq_cols), 0)
            qbd[:, sl] = jnp.where(((col // DH) % G) == row, q, 0.0).astype(bf)

        cp_w1().wait()
        cp_w3().wait()
        ga = jnp.dot(x8, w1_v[...], preferred_element_type=f32)
        up = jnp.dot(x8, w3_v[...], preferred_element_type=f32)
        hh = (ga * jax.nn.sigmoid(ga) * up).astype(bf)
        cp_w2().wait()
        b = jnp.dot(hh, w2_v[...], preferred_element_type=f32)[0:1]

        col = lax.broadcasted_iota(jnp.int32, (8, GR), 1)
        row = lax.broadcasted_iota(jnp.int32, (8, GR), 0)
        omsk = (col // DH) == row

        def group(g, carry):
            s = g % NBUF
            off = pl.multiple_of(g * GR, 128)
            cp_k(g, s).wait()
            sc = jnp.dot(qbd[:, pl.ds(off, GR)], kbuf[s], preferred_element_type=f32) * scale
            m = jnp.max(sc, axis=-1, keepdims=True)
            p = jnp.exp(sc - m)
            l = jnp.sum(p, axis=-1, keepdims=True)

            @pl.when(g + NBUF < NG)
            def _():
                cp_k(g + NBUF, s).start()

            cp_v(g, s).wait()
            o = lax.dot_general(p.astype(bf), vbuf[s], (((1,), (1,)), ((), ())),
                                preferred_element_type=f32)
            obd[:, pl.ds(off, GR)] = jnp.where(omsk, o / l, 0.0).astype(bf)

            @pl.when(g + NBUF < NG)
            def _():
                cp_v(g + NBUF, s).start()

            @pl.when(g + NBUF == NG)
            def _():
                for i in range(WO_CH):
                    cp_wo(i).start()

            return carry

        lax.fori_loop(0, NG, group, 0)

        acc = jnp.zeros((8, D), f32)
        for i in range(WO_CH):
            cp_wo(i).wait()
            sl = pl.ds(i * wo_rows, wo_rows)
            acc = acc + jnp.dot(obd[:, sl], wo_v[sl, :], preferred_element_type=f32)
        a = jnp.sum(acc, axis=0, keepdims=True)
        o_ref[0] = (gate * a + (1.0 - gate) * b).astype(o_ref.dtype)

    kt = jnp.swapaxes(A_k_cache, 2, 3).reshape(HD, SK)
    vt = jnp.swapaxes(A_v_cache, 2, 3).reshape(HD, SK)
    return pl.pallas_call(
        kernel,
        in_specs=[pl.BlockSpec(memory_space=pl.ANY)] * 9,
        out_specs=pl.BlockSpec(memory_space=pltpu.VMEM),
        out_shape=jax.ShapeDtypeStruct((1, 1, D), bf),
        scratch_shapes=[
            pltpu.VMEM((1, 1, D), bf), pltpu.VMEM((D,), bf),
            pltpu.VMEM((D, HD), bf), pltpu.VMEM((HD, D), bf),
            pltpu.VMEM((D, F), bf), pltpu.VMEM((D, F), bf), pltpu.VMEM((F, D), bf),
            pltpu.VMEM((NBUF, GR, W), bf), pltpu.VMEM((NBUF, GR, W), bf),
            pltpu.VMEM((8, HD), bf), pltpu.VMEM((8, HD), bf),
            pltpu.SemaphoreType.DMA((2,)), pltpu.SemaphoreType.DMA((WQ_CH,)),
            pltpu.SemaphoreType.DMA((WO_CH,)), pltpu.SemaphoreType.DMA((3,)),
            pltpu.SemaphoreType.DMA((NBUF,)), pltpu.SemaphoreType.DMA((NBUF,)),
        ],
        compiler_params=pltpu.CompilerParams(vmem_limit_bytes=100 * 1024 * 1024),
    )(A_x, kt, vt, A_wq, A_wo, B_w1, B_w3, B_w2, gate_w)
```

```python
import jax
import jax.numpy as jnp
from jax import lax
import jax.experimental.pallas as pl
import jax.experimental.pallas.tpu as pltpu

H = 32
DH = 192
G = 2
NBUF = 3
WO_MXU = (4608, 1024, 256)
WO_VPU = (128, 96, 32)


@jax.jit
def pallas_gated_mix__sliding_block_cached__glu_gated_swiglu__decode_kernel(
    A_x: jax.Array,
    A_k_cache: jax.Array,
    A_v_cache: jax.Array,
    A_wq: jax.Array,
    A_wo: jax.Array,
    B_x: jax.Array,
    B_w1: jax.Array,
    B_w3: jax.Array,
    B_w2: jax.Array,
    gate_w: jax.Array,
):
    del B_x
    D = A_x.shape[-1]
    F = B_w1.shape[-1]
    SK = A_k_cache.shape[2]
    W = min(4096, max(256, SK // 4))
    HD = H * DH
    GR = G * DH
    NG = H // G
    RV = sum(WO_VPU)
    assert sum(WO_MXU) + RV == HD and RV % 128 == 0 and D % 128 == 0
    scale = DH ** -0.5
    bf = jnp.bfloat16
    f32 = jnp.float32

    wo_chunks = []
    r0 = RV
    for n in WO_MXU:
        wo_chunks.append((r0, n))
        r0 += n
    r0 = 0
    for n in WO_VPU:
        wo_chunks.append((r0, n))
        r0 += n

    S_X, S_WQ, S_FFN, S_K = 0, 1, 2, 3
    S_V = S_K + NBUF
    S_WO = S_V + NBUF
    NSEM = S_WO + len(wo_chunks)

    def kernel(x_hbm, k_hbm, v_hbm, wq_hbm, wo_hbm, w1_hbm, w3_hbm, w2_hbm, gw_hbm, o_hbm,
               out_v, x_v, gw_v, wq_v, wo_v, w1_v, w3_v, w2_v, kbuf, vbuf, qbd, obd, ocol,
               osem):
        copy = pltpu.make_async_copy

        def cp_out():
            return copy(out_v, o_hbm, osem)

        def body(sem):
            def cp_small():
                return (copy(x_hbm, x_v, sem.at[S_X]), copy(gw_hbm, gw_v, sem.at[S_X]))

            def cp_wq():
                return copy(wq_hbm, wq_v, sem.at[S_WQ])

            def cp_ffn():
                return (copy(w1_hbm, w1_v, sem.at[S_FFN]), copy(w3_hbm, w3_v, sem.at[S_FFN]),
                        copy(w2_hbm, w2_v, sem.at[S_FFN]))

            def cp_wo(i):
                rows = pl.ds(*wo_chunks[i])
                return copy(wo_hbm.at[rows, :], wo_v.at[rows, :], sem.at[S_WO + i])

            def cp_k(g, s):
                return copy(k_hbm.at[pl.ds(g * GR, GR), pl.ds(SK - W, W)], kbuf.at[s],
                            sem.at[S_K + s])

            def cp_v(g, s):
                return copy(v_hbm.at[pl.ds(g * GR, GR), pl.ds(SK - W, W)], vbuf.at[s],
                            sem.at[S_V + s])

            cp_wq().start()
            for c in cp_small() + cp_ffn():
                c.start()
            for g in range(NBUF):
                cp_k(g, g).start()
                cp_v(g, g).start()

            cp_wq().wait()
            for c in cp_small():
                c.wait()
            x = x_v[0]
            x8 = jnp.broadcast_to(x, (8, D))
            gw = gw_v[...].reshape(1, D)
            gate = jax.nn.sigmoid(
                jnp.sum(x.astype(f32) * gw.astype(f32), axis=-1, keepdims=True))

            q = jnp.dot(x8, wq_v[...], preferred_element_type=f32)
            col = lax.broadcasted_iota(jnp.int32, (8, HD), 1)
            row = lax.broadcasted_iota(jnp.int32, (8, HD), 0)
            qbd[...] = jnp.where(((col // DH) % G) == row, q, 0.0).astype(bf)

            for c in cp_ffn():
                c.wait()
            ga = jnp.dot(x8, w1_v[...], preferred_element_type=f32)
            up = jnp.dot(x8, w3_v[...], preferred_element_type=f32)
            row_f = lax.broadcasted_iota(jnp.int32, (8, F), 0)
            hh = jnp.where(row_f == 0, ga * jax.nn.sigmoid(ga) * up, 0.0).astype(bf)
            acc = (1.0 - gate) * jnp.dot(hh, w2_v[...], preferred_element_type=f32)

            diag = (lax.broadcasted_iota(jnp.int32, (8, GR), 1) // DH
                    == lax.broadcasted_iota(jnp.int32, (8, GR), 0))

            def group(g, carry):
                s = g % NBUF
                cols = pl.ds(pl.multiple_of(g * GR, 128), GR)
                cp_k(g, s).wait()
                sc = jnp.dot(qbd[:, cols], kbuf[s], preferred_element_type=f32) * scale
                m = jnp.max(sc, axis=-1, keepdims=True)
                p = jnp.exp(sc - m)
                l = jnp.sum(p, axis=-1, keepdims=True)

                @pl.when(g + NBUF < NG)
                def _():
                    cp_k(g + NBUF, s).start()

                cp_v(g, s).wait()
                o = lax.dot_general(p.astype(bf), vbuf[s], (((1,), (1,)), ((), ())),
                                    preferred_element_type=f32)
                obd[:, cols] = jnp.where(diag, o * (gate / l), 0.0).astype(bf)

                @pl.when(g + NBUF < NG)
                def _():
                    cp_v(g + NBUF, s).start()

                @pl.when(g + NBUF == NG)
                def _():
                    for i in range(len(wo_chunks)):
                        cp_wo(i).start()

                return carry

            lax.fori_loop(0, NG, group, 0)

            o0 = jnp.sum(obd[:, 0:RV].astype(f32), axis=0, keepdims=True)
            eye = (lax.broadcasted_iota(jnp.int32, (RV, RV), 0)
                   == lax.broadcasted_iota(jnp.int32, (RV, RV), 1))
            oc = jnp.sum(jnp.where(eye, jnp.broadcast_to(o0, (RV, RV)), 0.0),
                         axis=1, keepdims=True)
            ocol[...] = jnp.broadcast_to(oc, (RV, 128))

            for i, (start, n) in enumerate(wo_chunks):
                cp_wo(i).wait()
                if i < len(WO_MXU):
                    rows = pl.ds(start, n)
                    acc = acc + jnp.dot(obd[:, rows], wo_v[rows, :],
                                        preferred_element_type=f32)
                else:
                    for r in range(start, start + n, 8):
                        ob = jnp.concatenate([ocol[r:r + 8, :]] * (D // 128), axis=1)
                        acc = acc + wo_v[r:r + 8, :].astype(f32) * ob
            out_v[0] = jnp.sum(acc, axis=0, keepdims=True).astype(bf)
            cp_out().start()

        pl.run_scoped(body, pltpu.SemaphoreType.DMA((NSEM,)))
        cp_out().wait()

    kt = jnp.swapaxes(A_k_cache, 2, 3).reshape(HD, SK)
    vt = jnp.swapaxes(A_v_cache, 2, 3).reshape(HD, SK)
    return pl.pallas_call(
        kernel,
        in_specs=[pl.BlockSpec(memory_space=pl.ANY)] * 9,
        out_specs=pl.BlockSpec(memory_space=pl.ANY),
        out_shape=jax.ShapeDtypeStruct((1, 1, D), bf),
        scratch_shapes=[
            pltpu.VMEM((1, 1, D), bf),
            pltpu.VMEM((1, 1, D), bf),
            pltpu.VMEM((D,), bf),
            pltpu.VMEM((D, HD), bf),
            pltpu.VMEM((HD, D), bf),
            pltpu.VMEM((D, F), bf),
            pltpu.VMEM((D, F), bf),
            pltpu.VMEM((F, D), bf),
            pltpu.VMEM((NBUF, GR, W), bf),
            pltpu.VMEM((NBUF, GR, W), bf),
            pltpu.VMEM((8, HD), bf),
            pltpu.VMEM((8, HD), bf),
            pltpu.VMEM((RV, 128), f32),
            pltpu.SemaphoreType.DMA(()),
        ],
        compiler_params=pltpu.CompilerParams(vmem_limit_bytes=64 * 1024 * 1024),
    )(A_x, kt, vt, A_wq, A_wo, B_w1, B_w3, B_w2, gate_w)
```

```python
import jax
import jax.numpy as jnp
from jax import lax
import jax.experimental.pallas as pl
import jax.experimental.pallas.tpu as pltpu

H = 32
DH = 192
GR = 2 * DH
NG = H // 2
LAG = 16
SPIN_W = 5
SPIN_KV = 6


def _small_div(t, d, tmax):
    if isinstance(t, int):
        return t // d
    sh = 16
    m = ((1 << sh) + d - 1) // d
    assert all((x * m) >> sh == x // d for x in range(tmax))
    return lax.shift_right_logical(t * m, sh)


@jax.jit
def pallas_gated_mix__sliding_block_cached__glu_gated_swiglu__decode_kernel(
    A_x: jax.Array,
    A_k_cache: jax.Array,
    A_v_cache: jax.Array,
    A_wq: jax.Array,
    A_wo: jax.Array,
    B_x: jax.Array,
    B_w1: jax.Array,
    B_w3: jax.Array,
    B_w2: jax.Array,
    gate_w: jax.Array,
):
    del B_x
    D = A_x.shape[-1]
    F = B_w1.shape[-1]
    SK = A_k_cache.shape[2]
    W = min(4096, max(256, SK // 4))
    HD = H * DH
    assert (D, F, W) == (640, 1536, 4096)
    SLAB = HD // 4
    scale = DH ** -0.5
    bf = jnp.bfloat16
    f32 = jnp.float32
    NSEM = LAG + 4

    def kernel(x_hbm, k_hbm, v_hbm, wq_hbm, wo_hbm, w1_hbm, w3_hbm, w2_hbm, gw_hbm, o_hbm,
               out_v, x_v, gw_v, wq_v, wo_v, w1_v, w3_v, w2_v, kbuf, vbuf,
               q_v, obd, h_v, s_v, ocol, acc_v, cnt, osem):
        copy = pltpu.make_async_copy

        def cp_out():
            return copy(out_v, o_hbm, osem)

        def body(sem):
            def gsem(slot, half):
                return sem.at[LAG + 2 * slot + half]

            def col_piece(src, dst, ncb, i, s):
                ri = _small_div(i, ncb, 16 * ncb)
                ci = i - ri * ncb
                r = pl.ds(pl.multiple_of(ri * 8, 8), 8)
                c = pl.ds(pl.multiple_of(ci * 512, 128), 512)
                return copy(src.at[:, r, c], dst.at[:, r, c], s)

            def row_piece(src, dst, row, s):
                r = pl.ds(pl.multiple_of(row, 8), 8)
                return copy(src.at[:, r, :], dst.at[:, r, :], s)

            def kv_piece(src, dst, t, slot, b, r, s):
                r0 = pl.multiple_of((r & 1) * DH, 8)
                c0 = pl.multiple_of((8 * b + (r >> 1)) * 128, 128)
                return copy(src.at[pl.ds(t * GR + r0, DH), pl.ds(SK - W + c0, 128)],
                            dst.at[slot, pl.ds(r0, DH), pl.ds(c0, 128)], s)

            def ack_w1(r):
                col_piece(w1_hbm, w1_v, 3, 0, sem.at[r]).wait()

            def ack_w3(r):
                col_piece(w3_hbm, w3_v, 3, 0, sem.at[r]).wait()

            def ack_w2(r):
                row_piece(w2_hbm, w2_v, 0, sem.at[r]).wait()

            def ack_wo(r):
                row_piece(wo_hbm, wo_v, 0, sem.at[r]).wait()

            def ack_v(r):
                kv_piece(v_hbm, vbuf, 0, 0, 0, 0, sem.at[r]).wait()

            def wait_region(region, s):
                copy(region, region, s).wait()

            def idle_steps(lo, hi, ack, p1, p0, spins):
                def spin(i, c):
                    cnt[0] = cnt[0] + i
                    return c

                def step(r, c):
                    if ack is not None:
                        ack(r)
                    p1(r).start(priority=1)
                    p0(r).start(priority=0)
                    lax.fori_loop(0, spins, spin, 0)
                    return c

                lax.fori_loop(lo, hi, step, 0)

            def work_steps(lo, hi, ack, p1, p0, work, carry):
                issue, consume = work

                def pair(i, c):
                    r0, r1 = 2 * i, 2 * i + 1
                    ack(r0)
                    ack(r1)
                    p0(r0).start(priority=0)
                    p1(r0).start(priority=1)
                    t0, t1 = issue(r0), issue(r1)
                    p1(r1).start(priority=1)
                    p0(r1).start(priority=0)
                    return consume(r1, t1, consume(r0, t0, c))

                return lax.fori_loop(lo // 2, hi // 2, pair, carry)

            def tile(i, width=128):
                return pl.ds(pl.multiple_of(i * width, 128), width)

            def add(r, t, a):
                return a + t

            def cp_small():
                return (copy(x_hbm, x_v, gsem(1, 0)), copy(gw_hbm, gw_v, gsem(1, 0)))

            cnt[0] = 0
            wq_sem = gsem(1, 1)

            def a_p0(b):
                return lambda r: col_piece(wq_hbm, wq_v, 12, 16 * b + r, wq_sem)

            def a_p1(b):
                if b < 3:
                    return lambda r: col_piece(w1_hbm, w1_v, 3, 16 * b + r, sem.at[r])
                if b < 6:
                    return lambda r: col_piece(w3_hbm, w3_v, 3, 16 * (b - 3) + r, sem.at[r])
                if b < 9:
                    return lambda r: row_piece(w2_hbm, w2_v, 128 * (b - 6) + 8 * r, sem.at[r])
                return lambda r: row_piece(wo_hbm, wo_v, 1152 + 128 * (b - 9) + 8 * r, sem.at[r])

            a_ack = [None] + [ack_w1] * 3 + [ack_w3] * 3 + [ack_w2] * 3 + [ack_wo] * 2

            for b in range(7):
                idle_steps(0, 16, a_ack[b], a_p1(b), a_p0(b), SPIN_W)
                if b == 0:
                    for c in cp_small():
                        c.start()

            for c in cp_small():
                c.wait()
            x = x_v[0]
            x8 = jnp.broadcast_to(x, (8, D))
            gw = gw_v[...].reshape(1, D)
            gate = jax.nn.sigmoid(
                jnp.sum(x.astype(f32) * gw.astype(f32), axis=-1, keepdims=True))
            row0 = lax.broadcasted_iota(jnp.int32, (8, 128), 0) == 0

            for b in (7, 8):
                def h_pair(i, c, b=b):
                    cols = tile(6 * (b - 7) + i)
                    a_ack[b](2 * i)
                    a_ack[b](2 * i + 1)
                    a_p0(b)(2 * i).start(priority=0)
                    a_p1(b)(2 * i).start(priority=1)
                    ga = jnp.dot(x8, w1_v[:, :, cols].reshape(D, 128), preferred_element_type=f32)
                    up = jnp.dot(x8, w3_v[:, :, cols].reshape(D, 128), preferred_element_type=f32)
                    a_p1(b)(2 * i + 1).start(priority=1)
                    a_p0(b)(2 * i + 1).start(priority=0)
                    hh = ga * jax.nn.sigmoid(ga) * up * (1.0 - gate)
                    h_v[:, cols] = jnp.where(row0, hh, 0.0).astype(bf)
                    return c

                lax.fori_loop(0, 6, h_pair, 0)
                idle_steps(12, 16, a_ack[b], a_p1(b), a_p0(b), SPIN_W)
            idle_steps(0, 16, a_ack[9], a_p1(9), a_p0(9), SPIN_W)

            def w2_issue(r):
                s, rb = r & 3, r >> 2
                return jnp.dot(h_v[:, tile(3 * s + rb)], w2_v[s, tile(rb), :],
                               preferred_element_type=f32)

            acc_v[...] = work_steps(0, 12, a_ack[10], a_p1(10), a_p0(10), (w2_issue, add),
                                    jnp.zeros((8, D), f32))
            idle_steps(12, 16, a_ack[10], a_p1(10), a_p0(10), SPIN_W)
            idle_steps(0, 16, a_ack[11], a_p1(11), a_p0(11), SPIN_W)

            def v_p1(t, slot, b):
                return lambda r: kv_piece(v_hbm, vbuf, t, slot, b, r, sem.at[r])

            def k_p0(t, slot, b):
                return lambda r: kv_piece(k_hbm, kbuf, t, slot, b, r, gsem(slot, b // 2))

            def wait_k(slot, half):
                wait_region(kbuf.at[slot, :, pl.ds(half * (W // 2), W // 2)], gsem(slot, half))

            idle_steps(0, 16, ack_wo, v_p1(0, 0, 0), k_p0(0, 0, 0), SPIN_KV)
            wait_region(wq_v, wq_sem)
            for b in range(1, 4):
                def q_issue(r, b=b):
                    cols = tile(16 * (b - 1) + r)
                    return jnp.dot(x8, wq_v[:, :, cols].reshape(D, 128),
                                   preferred_element_type=f32)

                def q_store(r, t, c, b=b):
                    q_v[:, tile(16 * (b - 1) + r)] = t.astype(bf)
                    return c

                work_steps(0, 16, ack_v, v_p1(0, 0, b), k_p0(0, 0, b), (q_issue, q_store), 0)

            diag = (lax.broadcasted_iota(jnp.int32, (8, GR), 1) // DH
                    == lax.broadcasted_iota(jnp.int32, (8, GR), 0))
            eye = (lax.broadcasted_iota(jnp.int32, (128, 128), 0)
                   == lax.broadcasted_iota(jnp.int32, (128, 128), 1))

            def attention(g, slot, tw):
                gcols = tile(g, GR)
                qg = jnp.where(diag, q_v[:, gcols].astype(f32), 0.0).astype(bf)

                def qk(base):
                    def issue(r):
                        return jnp.dot(qg, kbuf[slot, :, tile(base + r, tw)],
                                       preferred_element_type=f32)

                    def consume(r, s, mx):
                        s = s * scale
                        s_v[:, tile(base + r, tw)] = s
                        return jnp.maximum(mx, s)

                    return issue, consume

                def pv(base, m):
                    def issue(r):
                        cols = tile(base + r, tw)
                        p = jnp.exp(s_v[:, cols] - m)
                        o = lax.dot_general(p.astype(bf), vbuf[slot, :, cols],
                                            (((1,), (1,)), ((), ())),
                                            preferred_element_type=f32)
                        return p, o

                    def consume(r, t, c):
                        return c[0] + t[0], c[1] + t[1]

                    return issue, consume

                def finish(c):
                    l = jnp.sum(c[0], axis=-1, keepdims=True)
                    o = jnp.where(diag, c[1] * (gate / l), 0.0).astype(bf)
                    obd[:, gcols] = o

                    def resident():
                        acc_v[...] += jnp.dot(o, wo_v[g >> 2, 1152:1536, :],
                                              preferred_element_type=f32)

                    def column_form():
                        o0 = jnp.broadcast_to(o[0:1, 0:128].astype(f32), (128, 128))
                        oc = jnp.sum(jnp.where(eye, o0, 0.0), axis=1, keepdims=True)
                        ocol[g >> 2] = jnp.broadcast_to(oc, (128, 128))

                    if isinstance(g, int):
                        assert g & 3 == 3
                        resident()
                    else:
                        pl.when((g & 3) == 3)(resident)
                        pl.when((g & 3) == 0)(column_form)

                mx0 = jnp.full((8, tw), -jnp.inf, f32)
                c0 = (jnp.zeros((8, tw), f32), jnp.zeros((8, GR), f32))
                return qk, pv, finish, mx0, c0

            def group(t, carry):
                slot = t & 1
                prev = 1 - slot
                qk, pv, finish, mx, c = attention(t - 1, prev, 128)
                wait_k(prev, 0)
                mx = work_steps(0, 16, ack_v, v_p1(t, slot, 0), k_p0(t, slot, 0), qk(0), mx)
                wait_k(prev, 1)
                mx = work_steps(0, 16, ack_v, v_p1(t, slot, 1), k_p0(t, slot, 1), qk(16), mx)
                m = jnp.max(mx, axis=-1, keepdims=True)
                c = work_steps(0, 16, ack_v, v_p1(t, slot, 2), k_p0(t, slot, 2), pv(0, m), c)
                c = work_steps(0, 16, ack_v, v_p1(t, slot, 3), k_p0(t, slot, 3), pv(16, m), c)
                finish(c)
                return carry

            lax.fori_loop(1, NG, group, 0)

            c_sem = [gsem(0, 0), gsem(0, 1), gsem(1, 0), gsem(1, 1)]

            def c_p0(b):
                return lambda r: row_piece(wo_hbm, wo_v, 128 + 128 * b + 8 * r, c_sem[b])

            def c_p1(b):
                return lambda r: row_piece(wo_hbm, wo_v, 640 + 128 * b + 8 * r, sem.at[r])

            def wait_c0(b):
                wait_region(wo_v.at[:, pl.ds(128 + 128 * b, 128), :], c_sem[b])

            def wo_dot(rb):
                def issue(r):
                    s = r & 3
                    return jnp.dot(obd[:, tile(s * (SLAB // 128) + rb)],
                                   wo_v[s, pl.ds(rb * 128, 128), :], preferred_element_type=f32)

                return issue, add

            last = (NG - 1) & 1
            qk, pv, finish, mx, c = attention(NG - 1, last, 256)
            wait_k(last, 0)
            mx = work_steps(0, 8, ack_v, c_p1(0), c_p0(0), qk(0), mx)
            wait_k(last, 1)
            mx = work_steps(8, 16, ack_v, c_p1(0), c_p0(0), qk(0), mx)
            m = jnp.max(mx, axis=-1, keepdims=True)
            c = work_steps(0, 16, ack_wo, c_p1(1), c_p0(1), pv(0, m), c)
            finish(c)
            acc = acc_v[...]
            wait_c0(0)
            acc = work_steps(0, 4, ack_wo, c_p1(2), c_p0(2), wo_dot(1), acc)
            acc = work_steps(4, 8, ack_wo, c_p1(2), c_p0(2), wo_dot(5), acc)
            idle_steps(8, 12, ack_wo, c_p1(2), c_p0(2), SPIN_W)
            wait_c0(1)
            acc = work_steps(12, 16, ack_wo, c_p1(2), c_p0(2), wo_dot(2), acc)
            acc = work_steps(0, 4, ack_wo, c_p1(3), c_p0(3), wo_dot(6), acc)
            idle_steps(4, 12, ack_wo, c_p1(3), c_p0(3), SPIN_W)
            wait_c0(2)
            acc = work_steps(12, 16, ack_wo, c_p1(3), c_p0(3), wo_dot(3), acc)

            def t_p0(r):
                return row_piece(wo_hbm, wo_v, 8 * r, c_sem[0])

            def t_p1(r):
                return row_piece(wo_hbm, wo_v, 64 + 8 * r, sem.at[r])

            def vpu_rows(a, r0):
                for s in range(4):
                    ob = jnp.concatenate([ocol[s, r0:r0 + 8, :]] * (D // 128), axis=1)
                    a = a + wo_v[s, r0:r0 + 8, :].astype(f32) * ob
                return a

            acc = work_steps(0, 4, ack_wo, t_p1, t_p0, wo_dot(7), acc)
            idle_steps(4, 8, ack_wo, t_p1, t_p0, SPIN_W)
            wait_c0(3)
            for s in range(4):
                acc = acc + wo_dot(4)[0](s)
            wait_region(wo_v.at[:, pl.ds(0, 64), :], c_sem[0])
            for r0 in range(0, 64, 8):
                acc = vpu_rows(acc, r0)
            for r in range(8, 16):
                ack_wo(r)
            for s in range(4):
                acc = acc + wo_dot(8)[0](s)
            for r in range(8):
                ack_wo(r)
                acc = vpu_rows(acc, 64 + 8 * r)
            out_v[0] = jnp.sum(acc, axis=0, keepdims=True).astype(bf)
            cp_out().start()

        pl.run_scoped(body, pltpu.SemaphoreType.DMA((NSEM,)))
        cp_out().wait()

    kt = jnp.swapaxes(A_k_cache, 2, 3).reshape(HD, SK)
    vt = jnp.swapaxes(A_v_cache, 2, 3).reshape(HD, SK)
    return pl.pallas_call(
        kernel,
        in_specs=[pl.BlockSpec(memory_space=pl.ANY)] * 9,
        out_specs=pl.BlockSpec(memory_space=pl.ANY),
        out_shape=jax.ShapeDtypeStruct((1, 1, D), bf),
        scratch_shapes=[
            pltpu.VMEM((1, 1, D), bf),
            pltpu.VMEM((1, 1, D), bf),
            pltpu.VMEM((D,), bf),
            pltpu.VMEM((5, 128, HD), bf),
            pltpu.VMEM((4, SLAB, D), bf),
            pltpu.VMEM((5, 128, F), bf),
            pltpu.VMEM((5, 128, F), bf),
            pltpu.VMEM((4, F // 4, D), bf),
            pltpu.VMEM((2, GR, W), bf),
            pltpu.VMEM((2, GR, W), bf),
            pltpu.VMEM((8, HD), bf),
            pltpu.VMEM((8, HD), bf),
            pltpu.VMEM((8, F), bf),
            pltpu.VMEM((8, W), f32),
            pltpu.VMEM((4, 128, 128), f32),
            pltpu.VMEM((8, D), f32),
            pltpu.SMEM((1,), jnp.int32),
            pltpu.SemaphoreType.DMA(()),
        ],
        compiler_params=pltpu.CompilerParams(vmem_limit_bytes=64 * 1024 * 1024),
    )(A_x, kt, vt, A_wq.reshape(5, 128, HD), A_wo.reshape(4, SLAB, D),
      B_w1.reshape(5, 128, F), B_w3.reshape(5, 128, F), B_w2.reshape(4, F // 4, D), gate_w)
```

```python
import jax
import jax.numpy as jnp
from jax import lax
import jax.experimental.pallas as pl
import jax.experimental.pallas.tpu as pltpu

H = 32
DH = 192
GR = 2 * DH
NG = H // 2
LAG = 8
GAP_W = 9
GAP_KV = 8

S_K, S_X, S_WQ, S_C, S_T0, S_T1, S_OUT, NSEM = LAG, LAG + 4, LAG + 5, LAG + 6, LAG + 10, \
    LAG + 11, LAG + 13, LAG + 14


def _small_div(t, d, tmax):
    if isinstance(t, int):
        return t // d
    sh = 16
    m = ((1 << sh) + d - 1) // d
    assert all((x * m) >> sh == x // d for x in range(tmax))
    return lax.shift_right_logical(t * m, sh)


def _aligned(start, size, align):
    if isinstance(start, int):
        return pl.ds(start, size)
    return pl.ds(pl.multiple_of(start, align), size)


def _tile(i, width=128):
    return _aligned(i * width, width, 128)


@jax.jit
def pallas_gated_mix__sliding_block_cached__glu_gated_swiglu__decode_kernel(
    A_x: jax.Array,
    A_k_cache: jax.Array,
    A_v_cache: jax.Array,
    A_wq: jax.Array,
    A_wo: jax.Array,
    B_x: jax.Array,
    B_w1: jax.Array,
    B_w3: jax.Array,
    B_w2: jax.Array,
    gate_w: jax.Array,
):
    del B_x
    D = A_x.shape[-1]
    F = B_w1.shape[-1]
    SK = A_k_cache.shape[2]
    W = min(4096, max(256, SK // 4))
    HD = H * DH
    assert (D, F, W) == (640, 1536, 4096)
    SLAB = HD // 4
    scale = DH ** -0.5
    bf = jnp.bfloat16
    f32 = jnp.float32

    def kernel(x_hbm, k_hbm, v_hbm, wq_hbm, wo_hbm, w1_hbm, w3_hbm, w2_hbm, gw_hbm, o_hbm,
               out_v, x_v, gw_v, wq_v, wo_v, w1_v, w3_v, w2_v, kbuf, vbuf,
               q_v, obd, h_v, s_v, ocol, acc_v, pace_v):
        copy = pltpu.make_async_copy

        def body(sem):
            def col_piece(src, dst, ncb, i, s):
                ri = _small_div(i, ncb, 16 * ncb)
                r, c = _aligned(ri * 8, 8, 8), _tile(i - ri * ncb, 512)
                return copy(src.at[:, r, c], dst.at[:, r, c], s)

            def row_piece(src, dst, row, n, s):
                r = _aligned(row, n, 8)
                return copy(src.at[:, r, :], dst.at[:, r, :], s)

            def kv_piece(src, dst, t, slot, ct, r0, n, s):
                return copy(src.at[_aligned(t * GR + r0, n, 8), _aligned(SK - W + ct * 128, 128, 128)],
                            dst.at[slot, pl.ds(r0, n), _tile(ct)], s)

            def wait_region(region, s):
                copy(region, region, s).wait()

            def pause(n):
                pace_v[...] = lax.fori_loop(0, n, lambda i, v: v * 0.5 + 1.0, pace_v[...])

            def idle_step(r, prev, p1, p0, gap):
                if prev is not None:
                    for c in prev(r):
                        c.wait()
                hi = p0(r)
                hi[0].start(priority=0)
                for c in p1(r):
                    c.start(priority=1)
                pause(gap)
                for c in hi[1:]:
                    c.start(priority=0)
                    pause(gap)

            def idle_steps(lo, hi, prev, p1, p0, gap):
                def step(r, carry):
                    idle_step(r, prev, p1, p0, gap)
                    return carry

                lax.fori_loop(lo, hi, step, 0)

            def work_steps(lo, hi, prev, p1, p0, work, carry):
                issue, consume = work

                def step(r, carry):
                    hi_c = p0(r)
                    hi_c[0].start(priority=0)
                    for c in prev(r):
                        c.wait()
                    for c in hi_c[1:-1]:
                        c.start(priority=0)
                        pause(2)
                    for c in p1(r):
                        c.start(priority=1)
                    t = issue(r)
                    hi_c[-1].start(priority=0)
                    return consume(r, t, carry)

                return lax.fori_loop(lo, hi, step, carry)

            def dot(a, b):
                return jnp.dot(a, b, preferred_element_type=f32)

            def cp_small():
                return (copy(x_hbm, x_v, sem.at[S_X]), copy(gw_hbm, gw_v, sem.at[S_X]))

            def a_p0(b):
                return lambda r: [col_piece(wq_hbm, wq_v, 12, 16 * b + 2 * r + j, sem.at[S_WQ])
                                  for j in range(2)]

            def a_p1(b):
                if b < 6:
                    return lambda r: [col_piece(w1_hbm, w1_v, 3, 8 * b + r, sem.at[r]),
                                      col_piece(w3_hbm, w3_v, 3, 8 * b + r, sem.at[r])]
                if b < 9:
                    return lambda r: [row_piece(w2_hbm, w2_v, 128 * (b - 6) + 16 * r, 16, sem.at[r])]
                return lambda r: [row_piece(wo_hbm, wo_v, 1152 + 128 * (b - 9) + 16 * r, 16,
                                            sem.at[r])]

            def a_idle(b, lo=0):
                idle_steps(lo, LAG, a_p1(b - 1) if b else None, a_p1(b), a_p0(b), GAP_W)

            def a_work(b, n, work, carry):
                carry = work_steps(0, n, a_p1(b - 1), a_p1(b), a_p0(b), work, carry)
                a_idle(b, n)
                return carry

            pace_v[...] = jnp.zeros(pace_v.shape, f32)
            idle_step(0, None, a_p1(0), a_p0(0), GAP_W + 3)
            a_idle(0, 1)
            for c in cp_small():
                c.start()
            for b in range(1, 7):
                a_idle(b)

            for c in cp_small():
                c.wait()
            x = x_v[0]
            x8 = jnp.broadcast_to(x, (8, D))
            gw = gw_v[...].reshape(1, D)
            gate = jax.nn.sigmoid(
                jnp.sum(x.astype(f32) * gw.astype(f32), axis=-1, keepdims=True))
            row0 = lax.broadcasted_iota(jnp.int32, (8, 128), 0) == 0

            for b in (7, 8):
                def h_issue(r, b=b):
                    cols = _tile(6 * (b - 7) + r)
                    return (dot(x8, w1_v[:, :, cols].reshape(D, 128)),
                            dot(x8, w3_v[:, :, cols].reshape(D, 128)))

                def h_store(r, t, carry, b=b):
                    ga, up = t
                    hh = ga * jax.nn.sigmoid(ga) * up * (1.0 - gate)
                    h_v[:, _tile(6 * (b - 7) + r)] = jnp.where(row0, hh, 0.0).astype(bf)
                    return carry

                a_work(b, 6, (h_issue, h_store), 0)
            a_idle(9)
            acc_v[...] = a_work(
                10, 4, (lambda r: dot(h_v[:, _tile(r, F // 4)], w2_v[r]), lambda r, t, a: a + t),
                jnp.zeros((8, D), f32))
            a_idle(11)

            def v_p1(t, slot, b):
                return lambda r: [kv_piece(v_hbm, vbuf, t, slot, 8 * b + r, 0, GR, sem.at[r])]

            def k_p0(t, slot, b):
                return lambda r: [kv_piece(k_hbm, kbuf, t, slot, 8 * b + r, 128 * j, 128,
                                           sem.at[S_K + 2 * slot + b // 2]) for j in range(3)]

            def wait_k(slot, half):
                wait_region(kbuf.at[slot, :, pl.ds(half * (W // 2), W // 2)],
                            sem.at[S_K + 2 * slot + half])

            idle_steps(0, LAG, a_p1(11), v_p1(0, 0, 0), k_p0(0, 0, 0), GAP_KV)
            wait_region(wq_v, sem.at[S_WQ])
            for b in range(1, 4):
                def q_issue(r, b=b):
                    return dot(x8, wq_v[:, :, _tile(8 * (b - 1) + r, 256)].reshape(D, 256))

                def q_store(r, t, carry, b=b):
                    q_v[:, _tile(8 * (b - 1) + r, 256)] = t.astype(bf)
                    return carry

                work_steps(0, LAG, v_p1(0, 0, b - 1), v_p1(0, 0, b), k_p0(0, 0, b),
                           (q_issue, q_store), 0)

            diag = (lax.broadcasted_iota(jnp.int32, (8, GR), 1) // DH
                    == lax.broadcasted_iota(jnp.int32, (8, GR), 0))
            eye = (lax.broadcasted_iota(jnp.int32, (128, 128), 0)
                   == lax.broadcasted_iota(jnp.int32, (128, 128), 1))

            def attention(g, slot, tw):
                gcols = _tile(g, GR)
                qg = jnp.where(diag, q_v[:, gcols].astype(f32), 0.0).astype(bf)

                def qk(base):
                    def issue(r):
                        return dot(qg, kbuf[slot, :, _tile(base + r, tw)])

                    def consume(r, s, mx):
                        s = s * scale
                        s_v[:, _tile(base + r, tw)] = s
                        return jnp.maximum(mx, s)

                    return issue, consume

                def pv(base, m):
                    def issue(r):
                        cols = _tile(base + r, tw)
                        p = jnp.exp(s_v[:, cols] - m)
                        o = lax.dot_general(p.astype(bf), vbuf[slot, :, cols],
                                            (((1,), (1,)), ((), ())),
                                            preferred_element_type=f32)
                        return p, o

                    def consume(r, t, c):
                        return c[0] + t[0], c[1] + t[1]

                    return issue, consume

                def finish(c):
                    l = jnp.sum(c[0], axis=-1, keepdims=True)
                    o = jnp.where(diag, c[1] * (gate / l), 0.0).astype(bf)
                    obd[:, gcols] = o

                    def resident():
                        acc_v[...] += dot(o, wo_v[g >> 2, 1152:1536, :])

                    def column_form():
                        o0 = jnp.broadcast_to(o[0:1, 0:128].astype(f32), (128, 128))
                        oc = jnp.sum(jnp.where(eye, o0, 0.0), axis=1, keepdims=True)
                        ocol[g >> 2] = jnp.broadcast_to(oc, (128, 128))

                    if isinstance(g, int):
                        assert g & 3 == 3
                        resident()
                    else:
                        pl.when((g & 3) == 3)(resident)
                        pl.when((g & 3) == 0)(column_form)

                mx0 = jnp.full((8, tw), -jnp.inf, f32)
                c0 = (jnp.zeros((8, tw), f32), jnp.zeros((8, GR), f32))
                return qk, pv, finish, mx0, c0

            def group(t, carry):
                slot = t & 1
                old = 1 - slot
                qk, pv, finish, mx, c = attention(t - 1, old, 256)
                v = [v_p1(t - 1, old, 3)] + [v_p1(t, slot, b) for b in range(4)]
                wait_k(old, 0)
                mx = work_steps(0, LAG, v[0], v[1], k_p0(t, slot, 0), qk(0), mx)
                wait_k(old, 1)
                mx = work_steps(0, LAG, v[1], v[2], k_p0(t, slot, 1), qk(8), mx)
                m = jnp.max(mx, axis=-1, keepdims=True)
                c = work_steps(0, LAG, v[2], v[3], k_p0(t, slot, 2), pv(0, m), c)
                c = work_steps(0, LAG, v[3], v[4], k_p0(t, slot, 3), pv(8, m), c)
                finish(c)
                return carry

            lax.fori_loop(1, NG, group, 0)

            def c_p0(b):
                return lambda r: [row_piece(wo_hbm, wo_v, 128 * (1 + b) + 16 * r + 8 * j, 8,
                                            sem.at[S_C + b]) for j in range(2)]

            def c_p1(b):
                return lambda r: [row_piece(wo_hbm, wo_v, 128 * (5 + b) + 16 * r, 16, sem.at[r])]

            def wait_c0(b):
                wait_region(wo_v.at[:, pl.ds(128 * (1 + b), 128), :], sem.at[S_C + b])

            def wo_block(s, rb):
                return dot(obd[:, _tile(s * (SLAB // 128) + rb)], wo_v[s, pl.ds(rb * 128, 128), :])

            def wo_dot(rb):
                return (lambda r: (wo_block(2 * (r & 1), rb), wo_block(2 * (r & 1) + 1, rb)),
                        lambda r, t, a: a + t[0] + t[1])

            last = (NG - 1) & 1
            qk, pv, finish, mx, c = attention(NG - 1, last, 512)
            wait_k(last, 0)
            mx = work_steps(0, 4, v_p1(NG - 1, last, 3), c_p1(0), c_p0(0), qk(0), mx)
            wait_k(last, 1)
            mx = work_steps(4, 8, v_p1(NG - 1, last, 3), c_p1(0), c_p0(0), qk(0), mx)
            m = jnp.max(mx, axis=-1, keepdims=True)
            c = work_steps(0, 8, c_p1(0), c_p1(1), c_p0(1), pv(0, m), c)
            finish(c)
            acc = acc_v[...]
            wait_c0(0)
            acc = work_steps(0, 2, c_p1(1), c_p1(2), c_p0(2), wo_dot(1), acc)
            acc = work_steps(2, 4, c_p1(1), c_p1(2), c_p0(2), wo_dot(5), acc)
            idle_steps(4, 6, c_p1(1), c_p1(2), c_p0(2), GAP_W)
            wait_c0(1)
            acc = work_steps(6, 8, c_p1(1), c_p1(2), c_p0(2), wo_dot(2), acc)
            acc = work_steps(0, 2, c_p1(2), c_p1(3), c_p0(3), wo_dot(6), acc)
            idle_steps(2, 6, c_p1(2), c_p1(3), c_p0(3), GAP_W)
            wait_c0(2)
            acc = work_steps(6, 8, c_p1(2), c_p1(3), c_p0(3), wo_dot(3), acc)

            def t_p0(r):
                return [row_piece(wo_hbm, wo_v, 16 * r + 8 * j, 8, sem.at[S_T0]) for j in range(2)]

            def t_p1(r):
                return [row_piece(wo_hbm, wo_v, 64 + 16 * r, 16, sem.at[r])]

            def t_last(r):
                rows = pl.ds(120, 8)
                return [row_piece(wo_hbm, wo_v, 112, 8, sem.at[r]),
                        copy(wo_hbm.at[0:3, rows, :], wo_v.at[0:3, rows, :], sem.at[S_T1]),
                        copy(wo_hbm.at[3:4, rows, :], wo_v.at[3:4, rows, :], sem.at[S_T1 + 1])]

            def vpu_rows(a, r0, slabs=range(4)):
                for s in slabs:
                    ob = jnp.concatenate([ocol[s, r0:r0 + 8, :]] * (D // 128), axis=1)
                    a = a + wo_v[s, r0:r0 + 8, :].astype(f32) * ob
                return a

            acc = work_steps(0, 2, c_p1(3), t_p1, t_p0, wo_dot(7), acc)
            idle_step(2, c_p1(3), t_p1, t_p0, GAP_W + 3)
            t_end = t_p0(3)
            idle_step(3, c_p1(3), t_last, lambda r: t_end[:1], GAP_W + 3)
            t_end[1].start(priority=0)
            wait_c0(3)
            for s in range(4):
                acc = acc + wo_block(s, 4)
            wait_region(wo_v.at[:, pl.ds(0, 64), :], sem.at[S_T0])
            for r0 in range(0, 64, 8):
                acc = vpu_rows(acc, r0)
            for r in range(4, 8):
                c_p1(3)(r)[0].wait()
            for s in range(4):
                acc = acc + wo_block(s, 8)
            for r in range(3):
                t_p1(r)[0].wait()
                acc = vpu_rows(vpu_rows(acc, 64 + 16 * r), 72 + 16 * r)
            fin = t_last(3)
            fin[0].wait()
            acc = vpu_rows(acc, 112)
            fin[1].wait()
            acc = vpu_rows(acc, 120, range(3))
            fin[2].wait()
            acc = vpu_rows(acc, 120, range(3, 4))
            out_v[0] = jnp.sum(acc, axis=0, keepdims=True).astype(bf)
            out = copy(out_v, o_hbm, sem.at[S_OUT])
            out.start()
            out.wait()

        pl.run_scoped(body, pltpu.SemaphoreType.DMA((NSEM,)))

    kt = jnp.swapaxes(A_k_cache, 2, 3).reshape(HD, SK)
    vt = jnp.swapaxes(A_v_cache, 2, 3).reshape(HD, SK)
    return pl.pallas_call(
        kernel,
        in_specs=[pl.BlockSpec(memory_space=pl.ANY)] * 9,
        out_specs=pl.BlockSpec(memory_space=pl.ANY),
        out_shape=jax.ShapeDtypeStruct((1, 1, D), bf),
        scratch_shapes=[
            pltpu.VMEM((1, 1, D), bf),
            pltpu.VMEM((1, 1, D), bf),
            pltpu.VMEM((D,), bf),
            pltpu.VMEM((5, 128, HD), bf),
            pltpu.VMEM((4, SLAB, D), bf),
            pltpu.VMEM((5, 128, F), bf),
            pltpu.VMEM((5, 128, F), bf),
            pltpu.VMEM((4, F // 4, D), bf),
            pltpu.VMEM((2, GR, W), bf),
            pltpu.VMEM((2, GR, W), bf),
            pltpu.VMEM((8, HD), bf),
            pltpu.VMEM((8, HD), bf),
            pltpu.VMEM((8, F), bf),
            pltpu.VMEM((8, W), f32),
            pltpu.VMEM((4, 128, 128), f32),
            pltpu.VMEM((8, D), f32),
            pltpu.VMEM((8, 128), f32),
        ],
        compiler_params=pltpu.CompilerParams(vmem_limit_bytes=64 * 1024 * 1024),
    )(A_x, kt, vt, A_wq.reshape(5, 128, HD), A_wo.reshape(4, SLAB, D),
      B_w1.reshape(5, 128, F), B_w3.reshape(5, 128, F), B_w2.reshape(4, F // 4, D), gate_w)
```

```python
import jax
import jax.numpy as jnp
from jax import lax
import jax.experimental.pallas as pl
import jax.experimental.pallas.tpu as pltpu

H = 32
DH = 192
GR = 2 * DH
NG = H // 2
LAG = 8
GAP_W = 9
GAP_KV = 4

S_K, S_X, S_WQ, S_C, S_T, S_OUT, NSEM = (LAG + i for i in (0, 4, 5, 6, 11, 13, 14))


def _small_div(t, d, tmax):
    if isinstance(t, int):
        return t // d
    sh = 16
    m = ((1 << sh) + d - 1) // d
    assert all((x * m) >> sh == x // d for x in range(tmax))
    return lax.shift_right_logical(t * m, sh)


def _aligned(start, size, align):
    if isinstance(start, int):
        return pl.ds(start, size)
    return pl.ds(pl.multiple_of(start, align), size)


def _tile(i, width=128):
    return _aligned(i * width, width, 128)


@jax.jit
def pallas_gated_mix__sliding_block_cached__glu_gated_swiglu__decode_kernel(
    A_x: jax.Array,
    A_k_cache: jax.Array,
    A_v_cache: jax.Array,
    A_wq: jax.Array,
    A_wo: jax.Array,
    B_x: jax.Array,
    B_w1: jax.Array,
    B_w3: jax.Array,
    B_w2: jax.Array,
    gate_w: jax.Array,
):
    del B_x
    D = A_x.shape[-1]
    F = B_w1.shape[-1]
    SK = A_k_cache.shape[2]
    W = min(4096, max(256, SK // 4))
    HD = H * DH
    assert (D, F, W) == (640, 1536, 4096)
    SLAB = HD // 4
    scale = DH ** -0.5
    bf = jnp.bfloat16
    f32 = jnp.float32

    def kernel(x_hbm, k_hbm, v_hbm, wq_hbm, wo_hbm, w1_hbm, w3_hbm, w2_hbm, gw_hbm, o_hbm,
               out_v, x_v, gw_v, wq_v, wo_v, w1_v, w3_v, w2_v, kbuf, vbuf,
               q_v, obd, h_v, s_v, ocol, acc_v, pace_v):
        copy = pltpu.make_async_copy

        def body(sem):
            def col_piece(src, dst, ncb, i, s):
                ri = _small_div(i, ncb, 16 * ncb)
                r, c = _aligned(ri * 8, 8, 8), _tile(i - ri * ncb, 512)
                return copy(src.at[:, r, c], dst.at[:, r, c], s)

            def row_piece(src, dst, row, n, s):
                r = _aligned(row, n, 8)
                return copy(src.at[:, r, :], dst.at[:, r, :], s)

            def kv_pieces(src, dst, t, slot, b, r, s):
                return [copy(src.at[_aligned(t * GR + 96 * b, 96, 8),
                                    _aligned(SK - W + (4 * r + j) * 128, 128, 128)],
                             dst.at[slot, pl.ds(96 * b, 96), _tile(4 * r + j)], s)
                        for j in range(4)]

            def wait_region(region, s):
                copy(region, region, s).wait()

            def pause(n):
                pace_v[...] = lax.fori_loop(0, n, lambda i, v: v * 0.5 + 1.0, pace_v[...])

            def idle_step(r, prev, p1, p0, gap):
                if prev is not None:
                    for c in prev(r):
                        c.wait()
                hi = p0(r)
                hi[0].start(priority=0)
                for c in p1(r):
                    c.start(priority=1)
                pause(gap)
                for c in hi[1:]:
                    c.start(priority=0)
                    pause(gap)

            def idle_steps(lo, hi, prev, p1, p0, gap):
                def step(r, carry):
                    idle_step(r, prev, p1, p0, gap)
                    return carry

                lax.fori_loop(lo, hi, step, 0)

            def work_steps(lo, hi, prev, p1, p0, work, carry):
                issue, consume = work

                def step(r, carry):
                    hi_c = p0(r)
                    hi_c[0].start(priority=0)
                    for c in prev(r):
                        c.wait()
                    if len(hi_c) > 2:
                        hi_c[1].start(priority=0)
                        pause(2)
                    t = issue(r)
                    for c in hi_c[2:-1]:
                        c.start(priority=0)
                    for c in p1(r):
                        c.start(priority=1)
                    hi_c[-1].start(priority=0)
                    return consume(r, t, carry)

                return lax.fori_loop(lo, hi, step, carry)

            def dot(a, b):
                return jnp.dot(a, b, preferred_element_type=f32)

            def cp_small():
                return (copy(x_hbm, x_v, sem.at[S_X]), copy(gw_hbm, gw_v, sem.at[S_X]))

            def a_p0(b):
                return lambda r: [col_piece(wq_hbm, wq_v, 12, 16 * b + 2 * r + j, sem.at[S_WQ])
                                  for j in range(2)]

            def a_p1(b):
                if b < 6:
                    return lambda r: [col_piece(w1_hbm, w1_v, 3, 8 * b + r, sem.at[r]),
                                      col_piece(w3_hbm, w3_v, 3, 8 * b + r, sem.at[r])]
                if b < 9:
                    return lambda r: [row_piece(w2_hbm, w2_v, 128 * (b - 6) + 16 * r, 16, sem.at[r])]
                return lambda r: [row_piece(wo_hbm, wo_v, 1152 + 128 * (b - 9) + 16 * r, 16,
                                            sem.at[r])]

            def a_idle(b, lo=0):
                idle_steps(lo, LAG, a_p1(b - 1) if b else None, a_p1(b), a_p0(b), GAP_W)

            def a_work(b, n, work, carry):
                carry = work_steps(0, n, a_p1(b - 1), a_p1(b), a_p0(b), work, carry)
                a_idle(b, n)
                return carry

            pace_v[...] = jnp.zeros(pace_v.shape, f32)
            idle_step(0, None, a_p1(0), a_p0(0), GAP_W + 3)
            a_idle(0, 1)
            for c in cp_small():
                c.start()
            for b in range(1, 7):
                a_idle(b)

            for c in cp_small():
                c.wait()
            x = x_v[0]
            x8 = jnp.broadcast_to(x, (8, D))
            gw = gw_v[...].reshape(1, D)
            gate = jax.nn.sigmoid(
                jnp.sum(x.astype(f32) * gw.astype(f32), axis=-1, keepdims=True))
            row0 = lax.broadcasted_iota(jnp.int32, (8, 128), 0) == 0

            for b in (7, 8):
                def h_issue(r, b=b):
                    cols = _tile(6 * (b - 7) + r)
                    return (dot(x8, w1_v[:, :, cols].reshape(D, 128)),
                            dot(x8, w3_v[:, :, cols].reshape(D, 128)))

                def h_store(r, t, carry, b=b):
                    ga, up = t
                    hh = ga * jax.nn.sigmoid(ga) * up * (1.0 - gate)
                    h_v[:, _tile(6 * (b - 7) + r)] = jnp.where(row0, hh, 0.0).astype(bf)
                    return carry

                a_work(b, 6, (h_issue, h_store), 0)
            a_idle(9)
            acc_v[...] = a_work(
                10, 4, (lambda r: dot(h_v[:, _tile(r, F // 4)], w2_v[r]), lambda r, t, a: a + t),
                jnp.zeros((8, D), f32))
            a_idle(11)

            def v_p1(t, slot, b):
                return lambda r: kv_pieces(v_hbm, vbuf, t, slot, b, r, sem.at[r])

            def k_p0(t, slot, b):
                return lambda r: kv_pieces(k_hbm, kbuf, t, slot, b, r,
                                           sem.at[S_K + 2 * slot + b // 2])

            def wait_k(slot, hh):
                wait_region(kbuf.at[slot, pl.ds(hh * DH, DH), :], sem.at[S_K + 2 * slot + hh])

            idle_steps(0, LAG, a_p1(11), v_p1(0, 0, 0), k_p0(0, 0, 0), GAP_KV)
            wait_region(wq_v, sem.at[S_WQ])
            for b in range(1, 4):
                def q_issue(r, b=b):
                    return dot(x8, wq_v[:, :, _tile(8 * (b - 1) + r, 256)].reshape(D, 256))

                def q_store(r, t, carry, b=b):
                    q_v[:, _tile(8 * (b - 1) + r, 256)] = t.astype(bf)
                    return carry

                work_steps(0, LAG, v_p1(0, 0, b - 1), v_p1(0, 0, b), k_p0(0, 0, b),
                           (q_issue, q_store), 0)

            diag = (lax.broadcasted_iota(jnp.int32, (8, GR), 1) // DH
                    == lax.broadcasted_iota(jnp.int32, (8, GR), 0))
            eye = (lax.broadcasted_iota(jnp.int32, (128, 128), 0)
                   == lax.broadcasted_iota(jnp.int32, (128, 128), 1))

            def attention(g, slot, tw):
                gcols = _tile(g, GR)
                qg = jnp.where(diag, q_v[:, gcols].astype(f32), 0.0).astype(bf)

                def qk(hh, base):
                    qh = qg[:, hh * DH:(hh + 1) * DH]

                    def issue(r):
                        return dot(qh, kbuf[slot, hh * DH:(hh + 1) * DH, _tile(base + r, 2 * tw)])

                    def consume(r, s, mx):
                        cols = _tile(base + r, 2 * tw)
                        s = s * scale
                        if hh == 0:
                            s_v[:, cols] = s
                            return mx
                        s = s + s_v[:, cols]
                        s_v[:, cols] = s
                        return jnp.maximum(mx, jnp.maximum(s[:, :tw], s[:, tw:]))

                    return issue, consume

                def pv(base, m):
                    def issue(r):
                        cols = _tile(base + r, tw)
                        p = jnp.exp(s_v[:, cols] - m)
                        o = lax.dot_general(p.astype(bf), vbuf[slot, :, cols],
                                            (((1,), (1,)), ((), ())),
                                            preferred_element_type=f32)
                        return p, o

                    def consume(r, t, c):
                        return c[0] + t[0], c[1] + t[1]

                    return issue, consume

                def finish(c):
                    l = jnp.sum(c[0], axis=-1, keepdims=True)
                    o = jnp.where(diag, c[1] * (gate / l), 0.0).astype(bf)
                    obd[:, gcols] = o

                    def resident():
                        acc_v[...] += dot(o, wo_v[g >> 2, 1152:1536, :])

                    def column_form():
                        o0 = jnp.broadcast_to(o[0:1, 0:128].astype(f32), (128, 128))
                        oc = jnp.sum(jnp.where(eye, o0, 0.0), axis=1, keepdims=True)
                        ocol[g >> 2] = jnp.broadcast_to(oc, (128, 128))

                    if not isinstance(g, int):
                        pl.when((g & 3) == 3)(resident)
                        pl.when((g & 3) == 0)(column_form)

                mx0 = jnp.full((8, tw), -jnp.inf, f32)
                c0 = (jnp.zeros((8, tw), f32), jnp.zeros((8, GR), f32))
                return qk, pv, finish, mx0, c0

            def group(t, carry):
                slot = t & 1
                old = 1 - slot
                qk, pv, finish, mx, c = attention(t - 1, old, 256)
                v = [v_p1(t - 1, old, 3)] + [v_p1(t, slot, b) for b in range(4)]
                wait_k(old, 0)
                mx = work_steps(0, LAG, v[0], v[1], k_p0(t, slot, 0), qk(0, 0), mx)
                wait_k(old, 1)
                mx = work_steps(0, LAG, v[1], v[2], k_p0(t, slot, 1), qk(1, 0), mx)
                m = jnp.max(mx, axis=-1, keepdims=True)
                c = work_steps(0, LAG, v[2], v[3], k_p0(t, slot, 2), pv(0, m), c)
                c = work_steps(0, LAG, v[3], v[4], k_p0(t, slot, 3), pv(8, m), c)
                finish(c)
                return carry

            lax.fori_loop(1, NG, group, 0)

            def c_p0(b):
                if b < 2:
                    def pieces(r):
                        js = [24 * b + 3 * r + i for i in range(3)]
                        return [row_piece(wo_hbm, wo_v, 128 + 8 * j, 8, sem.at[S_C + (j >> 4)])
                                for j in js]
                    return pieces
                rb = (4, 8)[b - 2]
                return lambda r: [row_piece(wo_hbm, wo_v, 128 * rb + 16 * r + 8 * i, 8,
                                            sem.at[S_C + b + 1]) for i in range(2)]

            def c_p1(b):
                rb = (5, 6, 7, 0)[b]
                return lambda r: [row_piece(wo_hbm, wo_v, 128 * rb + 16 * r, 16, sem.at[r])]

            def c_last(r):
                rows = pl.ds(120, 8)
                return [row_piece(wo_hbm, wo_v, 112, 8, sem.at[r]),
                        copy(wo_hbm.at[0:3, rows, :], wo_v.at[0:3, rows, :], sem.at[S_T]),
                        copy(wo_hbm.at[3:4, rows, :], wo_v.at[3:4, rows, :], sem.at[S_T + 1])]

            def wait_c0(rb):
                wait_region(wo_v.at[:, pl.ds(128 * rb, 128), :],
                            sem.at[S_C + (1, 2, 3, 4, 8).index(rb)])

            def wo_block(s, rb):
                return dot(obd[:, _tile(s * (SLAB // 128) + rb)], wo_v[s, pl.ds(rb * 128, 128), :])

            def add_all(r, t, a):
                for u in t:
                    a = a + u
                return a

            def wo_dot(rb):
                return (lambda r: (wo_block(2 * (r & 1), rb), wo_block(2 * (r & 1) + 1, rb)),
                        add_all)

            def vpu_rows(a, r0, slabs=range(4)):
                for s in slabs:
                    ob = jnp.concatenate([ocol[s, r0:r0 + 8, :]] * (D // 128), axis=1)
                    a = a + wo_v[s, r0:r0 + 8, :].astype(f32) * ob
                return a

            last = (NG - 1) & 1
            qk, pv, finish, mx, c = attention(NG - 1, last, 512)
            wait_k(last, 0)
            mx = work_steps(0, 4, v_p1(NG - 1, last, 3), c_p1(0), c_p0(0), qk(0, 0), mx)
            wait_k(last, 1)
            mx = work_steps(4, 8, v_p1(NG - 1, last, 3), c_p1(0), c_p0(0), qk(1, -4), mx)
            m = jnp.max(mx, axis=-1, keepdims=True)
            c = work_steps(0, 8, c_p1(0), c_p1(1), c_p0(1), pv(0, m), c)
            finish(c)
            acc = acc_v[...]
            blk2 = (c_p1(1), c_p1(2), c_p0(2))
            blk3 = (c_p1(2), c_p1(3), c_p0(3))
            wait_c0(1)
            acc = work_steps(0, 2, *blk2, wo_dot(1), acc)
            acc = work_steps(2, 4, *blk2, wo_dot(5), acc)
            wait_c0(2)
            acc = work_steps(4, 6, *blk2, wo_dot(2), acc)
            wait_c0(3)
            acc = work_steps(6, 8, *blk2, wo_dot(3), acc)
            acc = work_steps(0, 2, *blk3, wo_dot(6), acc)
            acc = work_steps(2, 3, *blk3, (lambda r: (wo_block(3, 9), wo_block(3, 10)), add_all), acc)
            acc = work_steps(3, 4, *blk3, (lambda r: (wo_block(3, 11),), add_all), acc)
            wait_c0(4)
            acc = work_steps(4, 6, *blk3, wo_dot(4), acc)
            idle_step(6, *blk3, GAP_W + 3)
            c_end = c_p0(3)(7)
            idle_step(7, c_p1(2), c_last, lambda r: c_end[:1], GAP_W + 3)
            c_end[1].start(priority=0)
            for s in range(4):
                acc = acc + wo_block(s, 7)
            for r in range(2):
                c_p1(3)(r)[0].wait()
                acc = vpu_rows(vpu_rows(acc, 16 * r), 16 * r + 8)
            wait_c0(8)
            for s in range(4):
                acc = acc + wo_block(s, 8)
            for r in range(2, 7):
                c_p1(3)(r)[0].wait()
                acc = vpu_rows(vpu_rows(acc, 16 * r), 16 * r + 8)
            fin = c_last(7)
            fin[0].wait()
            acc = vpu_rows(acc, 112)
            fin[1].wait()
            acc = vpu_rows(acc, 120, range(3))
            fin[2].wait()
            acc = vpu_rows(acc, 120, range(3, 4))
            out_v[0] = jnp.sum(acc, axis=0, keepdims=True).astype(bf)
            out = copy(out_v, o_hbm, sem.at[S_OUT])
            out.start()
            out.wait()

        pl.run_scoped(body, pltpu.SemaphoreType.DMA((NSEM,)))

    kt = jnp.swapaxes(A_k_cache, 2, 3).reshape(HD, SK)
    vt = jnp.swapaxes(A_v_cache, 2, 3).reshape(HD, SK)
    return pl.pallas_call(
        kernel,
        in_specs=[pl.BlockSpec(memory_space=pl.ANY)] * 9,
        out_specs=pl.BlockSpec(memory_space=pl.ANY),
        out_shape=jax.ShapeDtypeStruct((1, 1, D), bf),
        scratch_shapes=[
            pltpu.VMEM((1, 1, D), bf),
            pltpu.VMEM((1, 1, D), bf),
            pltpu.VMEM((D,), bf),
            pltpu.VMEM((5, 128, HD), bf),
            pltpu.VMEM((4, SLAB, D), bf),
            pltpu.VMEM((5, 128, F), bf),
            pltpu.VMEM((5, 128, F), bf),
            pltpu.VMEM((4, F // 4, D), bf),
            pltpu.VMEM((2, GR, W), bf),
            pltpu.VMEM((2, GR, W), bf),
            pltpu.VMEM((8, HD), bf),
            pltpu.VMEM((8, HD), bf),
            pltpu.VMEM((8, F), bf),
            pltpu.VMEM((8, W), f32),
            pltpu.VMEM((4, 128, 128), f32),
            pltpu.VMEM((8, D), f32),
            pltpu.VMEM((8, 128), f32),
        ],
        compiler_params=pltpu.CompilerParams(vmem_limit_bytes=64 * 1024 * 1024),
    )(A_x, kt, vt, A_wq.reshape(5, 128, HD), A_wo.reshape(4, SLAB, D),
      B_w1.reshape(5, 128, F), B_w3.reshape(5, 128, F), B_w2.reshape(4, F // 4, D), gate_w)
```
